```python
import os as _os
_os.environ.setdefault("JAX_PLATFORMS", "cpu")
import jax
import jax.numpy as jnp

def _softmax(x, axis=-1):
    return jax.nn.softmax(x, axis=axis)
def _gelu(x):
    return jax.nn.gelu(x, approximate=True)
def _silu(x):
    return jax.nn.silu(x)
def _sigmoid(x):
    return jax.nn.sigmoid(x)
def _layernorm(x, axis=-1, eps=1e-5):
    m = jnp.mean(x, axis=axis, keepdims=True)
    v = jnp.var(x, axis=axis, keepdims=True)
    return (x - m) / jnp.sqrt(v + eps)
def _scatter_add(tgt, idx, src, axis=0):
    return tgt.at[idx].add(src)
def _segment_sum(src, seg, n):
    return jax.ops.segment_sum(src, seg, n)
class _Rng:
    def __init__(self, key):
        self._k = key
    def _next(self):
        self._k, sub = jax.random.split(self._k)
        return sub
    def normal(self, shape):
        return jax.random.normal(self._next(), shape, dtype=jnp.bfloat16)
    def randint(self, lo, hi, shape):
        return jax.random.randint(self._next(), shape, lo, hi, dtype=jnp.int32)
    def uniform(self, shape, lo=0.0, hi=1.0):
        return jax.random.uniform(self._next(), shape, jnp.bfloat16, lo, hi)
    def permutation(self, n):
        return jax.random.permutation(self._next(), n)


kernel_name = 'interleave_layers__sliding_local_dilated__sliding_local_dilated__prompt'

def setup_inputs():
    _rng = _Rng(jax.random.key(int.from_bytes(__import__("os").urandom(4), "little")))
    _w = (lambda a: (lambda t: t.astype(jnp.bfloat16) if jnp.issubdtype(t.dtype, jnp.floating) else t)(jnp.asarray(a)))
    def _A_setup():
        B, S, D = 1, 2048, 1024
        return {
            "x": _w((lambda *s: _rng.normal(s) * 0.05)(B, S, D)),
            "wqkv": _w((lambda *s: _rng.normal(s) * 0.05)(D, 3 * D)),
            "wo": _w((lambda *s: _rng.normal(s) * 0.05)(D, D)),
        }
    _A_in = _A_setup()

    def _B_setup():
        B, S, D = 1, 2048, 1024
        return {
            "x": _w((lambda *s: _rng.normal(s) * 0.05)(B, S, D)),
            "wqkv": _w((lambda *s: _rng.normal(s) * 0.05)(D, 3 * D)),
            "wo": _w((lambda *s: _rng.normal(s) * 0.05)(D, D)),
        }
    _B_in = _B_setup()

    return {
        "A_x": _A_in["x"],
        "A_wqkv": _A_in["wqkv"],
        "A_wo": _A_in["wo"],
        "B_x": _B_in["x"],
        "B_wqkv": _B_in["wqkv"],
        "B_wo": _B_in["wo"],
    }

def reference(A_x, A_wqkv, A_wo, B_x, B_wqkv, B_wo):
    def _A_ref(x, wqkv, wo):
        B, S, D = x.shape
        H = 32; Dh = D // H
        W, dil = 8, 2
        qkv = (lambda x, *d: x.transpose(*d))((x @ wqkv).reshape(B, S, 3, H, Dh), 2, 0, 3, 1, 4)
        q, k, v = qkv[0], qkv[1], qkv[2]
        scale = Dh ** -0.5
        pos = jnp.arange(S)
        off = jnp.arange(W) * dil
        idx = pos[:, None] - off[None, :]
        mask = idx >= 0
        idx_c = jnp.where(mask, idx, 0).reshape(-1)
        kg = k[:, :, idx_c, :].reshape(B, H, S, W, Dh)
        vg = v[:, :, idx_c, :].reshape(B, H, S, W, Dh)
        logits = jnp.einsum("bhsd,bhswd->bhsw", q, kg) * scale
        logits = jnp.where(mask[None, None, :, :], logits, -1e9)
        attn = _softmax(logits, axis=-1)
        o = jnp.einsum("bhsw,bhswd->bhsd", attn, vg)
        return (lambda x, *d: x.transpose(*d))(o, 0, 2, 1, 3).reshape(B, S, D) @ wo

    def _B_ref(x, wqkv, wo):
        B, S, D = x.shape
        H = 32; Dh = D // H
        W, dil = 8, 2
        qkv = (lambda x, *d: x.transpose(*d))((x @ wqkv).reshape(B, S, 3, H, Dh), 2, 0, 3, 1, 4)
        q, k, v = qkv[0], qkv[1], qkv[2]
        scale = Dh ** -0.5
        pos = jnp.arange(S)
        off = jnp.arange(W) * dil
        idx = pos[:, None] - off[None, :]
        mask = idx >= 0
        idx_c = jnp.where(mask, idx, 0).reshape(-1)
        kg = k[:, :, idx_c, :].reshape(B, H, S, W, Dh)
        vg = v[:, :, idx_c, :].reshape(B, H, S, W, Dh)
        logits = jnp.einsum("bhsd,bhswd->bhsw", q, kg) * scale
        logits = jnp.where(mask[None, None, :, :], logits, -1e9)
        attn = _softmax(logits, axis=-1)
        o = jnp.einsum("bhsw,bhswd->bhsd", attn, vg)
        return (lambda x, *d: x.transpose(*d))(o, 0, 2, 1, 3).reshape(B, S, D) @ wo

    x = A_x
    x = x + _A_ref(_layernorm(x, axis=-1), A_wqkv, A_wo)
    x = x + _B_ref(_layernorm(x, axis=-1), B_wqkv, B_wo)
    x = x + _A_ref(_layernorm(x, axis=-1), A_wqkv, A_wo)
    x = x + _B_ref(_layernorm(x, axis=-1), B_wqkv, B_wo)
    return x
```

```python
import functools
import math
import jax
import jax.numpy as jnp
from jax import lax
import jax.experimental.pallas as pl
import jax.experimental.pallas.tpu as pltpu

S, D = 2048, 1024
H, DH, W, DIL = 32, 32, 8, 2
NL = 4
LANES = 128
NB = D // LANES
HALO = 16
EPS = 1e-5
SCALE = DH ** -0.5
BF, F32, I32 = jnp.bfloat16, jnp.float32, jnp.int32


def _select_network(skew, g):
    n = len(skew)
    cur = [skew[(-b) % n] for b in range(n)]
    bit = 1
    while bit < n:
        m = (g & bit) != 0
        cur = [jnp.where(m, cur[(b - bit) % n], cur[b]) for b in range(n)]
        bit *= 2
    return cur


def _swap_granules(blocks, axis, gran):
    n = len(blocks)
    size = blocks[0].shape[axis]
    g = lax.broadcasted_iota(I32, blocks[0].shape, axis) // gran
    skew = [blocks[a] if a == 0 else pltpu.roll(blocks[a], a * gran, axis) for a in range(n)]
    cur = _select_network(skew, g)
    return [cur[b] if b == 0 else pltpu.roll(cur[b], size - b * gran, axis) for b in range(n)]


def _unpack(x):
    return tuple(pltpu.unpack_elementwise(x, index=i, packed_dtype=BF, unpacked_dtype=F32) for i in range(2))


def _pack(even, odd):
    return pltpu.bitcast(pltpu.pack_elementwise([even, odd], packed_dtype=BF), I32)


def _strassen_lhs(a11, a12, a21, a22):
    return a11 + a22, a21 + a22, a11, a22, a11 + a12, a21 - a11, a12 - a22


def _strassen_rhs(b11, b12, b21, b22):
    f11, f12, f21, f22 = map(_unpack, (b11, b12, b21, b22))
    add = lambda u, v: _pack(u[0] + v[0], u[1] + v[1])
    sub = lambda u, v: _pack(u[0] - v[0], u[1] - v[1])
    return add(f11, f22), b11, sub(f12, f22), sub(f21, f11), b22, add(f11, f12), add(f21, f22)


def _tree(op, xs):
    while len(xs) > 1:
        xs = [op(xs[i], xs[i + 1]) if i + 1 < len(xs) else xs[i] for i in range(0, len(xs), 2)]
    return xs[0]


def _merge(*streams):
    items = []
    for si, st in enumerate(streams):
        for i, f in enumerate(st):
            items.append(((i + (0.0 if si == 0 else 0.5)) / len(st), si, f))
    return [f for _, _, f in sorted(items, key=lambda z: z[:2])]


def _interleave(*streams):
    for f in _merge(*streams):
        f()


def _skewed(gens, nphase, dist=1):
    out = []
    for rnd in range(len(gens) + (nphase - 1) * dist):
        for p in range(nphase):
            i = rnd - p * dist
            if 0 <= i < len(gens):
                out.append(functools.partial(next, gens[i], None))
    return out


T = 256
R = 8
G = 16
PG = 16
NT = S // T
NSTEP = NL * NT
NG = T // R
NCB = NB // 2
WCH = NB // 2
WR = D // WCH
NACC = 2
ESPLIT = 2
WINDOW, AHEAD = 3, 4
P = functools.partial


def make_kernel():
    def kernel(x_hbm, wqkv_a, wo_a, wqkv_b, wo_b, out_hbm,
               xio, xres, wqkv_raw, wo_raw, wqkv_s, wo_s, h_s, o_s, of_s, acc_s, q_s, k_s, v_s,
               sem_x, sem_a, sem_b, sem_wo, sem_o):
        def x_copy(t):
            return pltpu.make_async_copy(x_hbm.at[pl.ds(t * T, T)], xio.at[pl.ds(t * T, T)], sem_x.at[t])

        def out_copy(t, part=0, nparts=1):
            rows = pl.ds(t * T + part * (T // nparts), T // nparts)
            return pltpu.make_async_copy(xio.at[rows], out_hbm.at[rows], sem_o.at[t + part])

        def wa_copy(p, i):
            rows, cols = pl.ds(i * WR, WR), pl.ds(p * D, D)
            return pltpu.make_async_copy(wqkv_a.at[rows, cols], wqkv_raw.at[0, rows, cols], sem_a.at[p * WCH + i])

        def woa_copy(i):
            rows = pl.ds(i * (D // 2), D // 2)
            return pltpu.make_async_copy(wo_a.at[rows], wo_raw.at[0, rows], sem_wo.at[i])

        def b_copies(i):
            out = []
            for half in range(2):
                rows = pl.ds(pl.multiple_of(i // 2 * WR + half * LANES + i % 2 * (LANES // 2), LANES // 2), LANES // 2)
                out.append(pltpu.make_async_copy(wqkv_b.at[rows], wqkv_raw.at[1, rows], sem_b.at[i % 2, half]))
            for a in range(4):
                rows = pl.ds(pl.multiple_of((i // 4 * 4 + a) * LANES + i % 4 * DH, DH), DH)
                out.append(pltpu.make_async_copy(wo_b.at[rows], wo_raw.at[1, rows], sem_b.at[i % 2, 2 + a]))
            return out

        def permute_group(ws, p, kk, r):
            skew = []
            for half in range(2):
                src = pl.ds(pl.multiple_of(kk * WR + half * LANES + r, PG), PG)
                blk = [pltpu.bitcast(wqkv_raw[ws, src, pl.ds(p * D + j * LANES, LANES)], I32) for j in range(NB)]
                skew.append([blk[j] if j == 0 else pltpu.roll(blk[j], 4 * j, 1) for j in range(NB)])
            yield
            out = []
            for half in range(2):
                cur = _select_network(skew[half], lax.broadcasted_iota(I32, (PG // 2, LANES), 1) // 4)
                out.append([cur[c] if c == 0 else pltpu.roll(cur[c], LANES - 4 * c, 1) for c in range(NB)])
            yield
            dst = pl.ds(pl.multiple_of((kk * LANES + r) // 2, PG // 2), PG // 2)
            for cb in range(NB // 2):
                ops = _strassen_rhs(out[0][cb], out[0][NB // 2 + cb], out[1][cb], out[1][NB // 2 + cb])
                for m in range(7):
                    wqkv_s[ws, p, m, dst, pl.ds(cb * LANES, LANES)] = ops[m]

        def permute_stream(items):
            return _skewed([permute_group(ws, p, kk, r0 + r) for ws, p, kk, r0, nrows in items
                            for r in range(0, nrows, PG)], 3, 2)

        def permute_wo(ws, i):
            j_hi, h_lo = i // 4, i % 4
            for c_hi in range(2):
                for cb in range(NB // 2):
                    out = []
                    for half in range(2):
                        cols = pl.ds(half * (D // 2) + cb * LANES, LANES)
                        src = [pltpu.bitcast(wo_raw[ws, pl.ds(pl.multiple_of(
                            (4 * j_hi + a) * LANES + h_lo * DH + c_hi * 16, 16), 16), cols], I32) for a in range(4)]
                        out.append(_swap_granules(src, 0, 2))
                    for e in range(2):
                        dst = pl.ds(pl.multiple_of(
                            (2 * c_hi + e) * (LANES // 2) + h_lo * (DH // 2) + j_hi * 8, 8), 8)
                        ops = _strassen_rhs(out[0][2 * e], out[1][2 * e], out[0][2 * e + 1], out[1][2 * e + 1])
                        for m in range(7):
                            wo_s[ws, m, dst, pl.ds(cb * LANES, LANES)] = ops[m]

        def widen_x(t, dst=None):
            rows = pl.ds(pl.multiple_of(t * T, T), T)
            to = rows if dst is None else pl.ds(pl.multiple_of(dst * T, T), T)
            for b in range(NB):
                xres[b, to, :] = xio[rows, pl.ds(b * LANES, LANES)].astype(F32)

        def load_pairs(ref, row, b):
            return [[ref[b, pl.ds(row + rh * G + e, G // 2, stride=2), :] for e in range(2)] for rh in range(2)]

        def store_lhs(dst, i, block):
            for kk in range(NB // 2):
                y0, y1 = block(2 * kk), block(2 * kk + 1)
                even, odd = (_strassen_lhs(y0[0][e], y1[0][e], y0[1][e], y1[1][e]) for e in range(2))
                for m in range(7):
                    dst[m, pl.ds(i * (G // 2), G // 2), pl.ds(kk * LANES, LANES)] = _pack(even[m], odd[m])

        def ln_rows(dst, row0, i):
            x = [load_pairs(xres, row0 + i * 2 * G, b) for b in range(NB)]
            y = [[[None, None], [None, None]] for _ in range(NB)]
            for rh in range(2):
                for e in range(2):
                    xs = [x[b][rh][e] for b in range(NB)]
                    m = jnp.sum(_tree(jnp.add, xs), axis=-1, keepdims=True) * (1.0 / D)
                    xc = [v - m for v in xs]
                    var = jnp.sum(_tree(jnp.add, [v * v for v in xc]), axis=-1, keepdims=True) * (1.0 / D)
                    r = lax.rsqrt(var + EPS)
                    for b in range(NB):
                        y[b][rh][e] = xc[b] * r
            store_lhs(dst, i, lambda b: y[b])

        def matmul_chunk(lhs, rhs, c, emit, part, nparts):
            n = T // 2 // nparts
            c11, c12, c21, c22 = ((c % NACC, k, pl.ds(part * n, n), slice(None)) for k in range(4))

            def product(m):
                return jnp.dot(pltpu.bitcast(lhs[m, pl.ds(part * n // 2, n // 2), :], BF),
                               pltpu.bitcast(rhs(m, pl.ds(c * LANES, LANES)), BF), preferred_element_type=F32)

            def finish(rh, ch, y):
                for g in range(n // G):
                    emit((part * n // G + g) * 2 * G + rh * G, ch * (NB // 2) + c, y[g * G:(g + 1) * G])

            acc_s[c11] = product(0)
            yield
            y = product(1)
            acc_s[c21] = y
            acc_s[c22] = acc_s[c11] - y
            yield
            y = product(2)
            acc_s[c12] = y
            acc_s[c22] = acc_s[c22] + y
            yield
            y = product(3)
            acc_s[c11] = acc_s[c11] + y
            finish(1, 0, acc_s[c21] + y)
            yield
            y = product(4)
            acc_s[c11] = acc_s[c11] - y
            finish(0, 1, acc_s[c12] + y)
            yield
            finish(1, 1, acc_s[c22] + product(5))
            yield
            finish(0, 0, acc_s[c11] + product(6))
            yield

        def products(gen):
            return [P(next, gen, None) for _ in range(7)]

        def qkv_chunk(src, ws, slot, p, c):
            ref, off = ((q_s, 0), (k_s, HALO), (v_s, HALO))[p]

            def emit(row, blk, y):
                ref[slot, blk, pl.ds(off + row, G), :] = y
            return products(matmul_chunk(src, lambda m, cols: wqkv_s[ws, p, m, :, cols], c, emit, 0, 1))

        def fill_halo(slot, first):
            for b in range(NB):
                for ref in (k_s, v_s):
                    prev = ref[1 - slot, b, pl.ds(T, HALO), :]
                    ref[slot, b, pl.ds(0, HALO), :] = jnp.where(first, 0.0, prev)

        def zero_halo(slot):
            for b in range(NB):
                for ref in (k_s, v_s):
                    ref[slot, b, pl.ds(0, HALO), :] = jnp.zeros((HALO, LANES), F32)

        def attn_stream(slot, row0):
            HW = W // 2
            q, part = {}, {}
            p = [[None] * W for _ in range(NG)]
            e, inv = [None] * NG, [None] * NG

            def users(n):
                return [(g, off) for g, off in ((n, 0), (n + 1, HW)) if 0 <= g < NG]

            def exchange(x, k):
                odd = (lax.broadcasted_iota(I32, (R, LANES), 1) & k) != 0
                return jnp.where(odd, pltpu.roll(x, k, 1), pltpu.roll(x, LANES - k, 1))

            def scores(n, j):
                for g, _ in users(n):
                    if j == 0:
                        q[g] = [q_s[slot, b, pl.ds(g * R, R), :] for b in range(NB)]
                keys = [k_s[slot, b, pl.ds(HALO + n * R - j * DIL, R), :] for b in range(NB)]
                for g, off in users(n):
                    x = functools.reduce(jnp.add, [q[g][b] * keys[b] for b in range(NB)])
                    p[g][off + j] = (x, exchange(x, 1))

            def reduce(n, j):
                for g, off in users(n):
                    x = p[g][off + j][0] + p[g][off + j][1]
                    p[g][off + j] = (x, exchange(x, 2))

            def finish(n, j):
                for g, off in users(n):
                    w = off + j
                    x = p[g][w][0] + p[g][w][1]
                    if g * R < w * DIL:
                        pos = row0 + g * R + lax.broadcasted_iota(I32, (R, LANES), 0)
                        x = jnp.where(pos >= w * DIL, x, -1e9 / SCALE)
                    p[g][w] = x

            def softmax_exp(g):
                m = functools.reduce(jnp.maximum, p[g])
                e[g] = [jnp.exp2((x - m) * (SCALE * math.log2(math.e))) for x in p[g]]

            def softmax_norm(g):
                inv[g] = 1.0 / functools.reduce(jnp.add, e[g])

            def values(n, b):
                vals = [v_s[slot, b, pl.ds(HALO + n * R - j * DIL, R), :] for j in range(HW)]
                for g, off in users(n):
                    x = functools.reduce(jnp.add, [e[g][off + j] * vals[j] for j in range(HW)])
                    if off:
                        part[g, b] = x
                    else:
                        of_s[b, pl.ds(g * R, R), :] = (x + part.pop((g, b))) * inv[g]

            cuts = []
            chains = [(n, j) for n in range(-1, NG) for j in range(HW)]
            steps = [[P(f, *chains[i - k]) for k, f in enumerate((scores, reduce, finish))
                      if 0 <= i - k < len(chains)] for i in range(len(chains) + 2)]
            out = []
            for r in range(-1, NG + 3):
                g = r - 2
                n = g - 1
                now = [sum(steps[(r + 1) * HW:(r + 2) * HW], [])]
                if 0 <= g < NG:
                    now.append([P(softmax_exp, g), P(softmax_norm, g)])
                if -1 <= n < NG:
                    now[-1] = now[-1] + [P(values, n, b) for b in range(NB)]
                out += _merge(*now)
                if 0 <= n < NG and (n + 1) * R % (2 * G) == 0:
                    i = n * R // (2 * G)
                    out.append(P(store_lhs, o_s, i, P(load_pairs, of_s, i * 2 * G)))
                    cuts.append(len(out))
            return out, cuts

        def wo_chunk(ws, row0, c, narrow, part=0, nparts=1):
            def emit(row, blk, y):
                rows = pl.ds(pl.multiple_of(row0 + row, G), G)
                y = xres[blk, rows, :] + y
                xres[blk, rows, :] = y
                if narrow:
                    xio[rows, pl.ds(blk * LANES, LANES)] = y.astype(BF)
            return products(matmul_chunk(o_s, lambda m, cols: wo_s[ws, m, :, cols], c, emit, part, nparts))

        def ln_stream(dst, row0):
            return [P(ln_rows, dst, row0, i) for i in range(T // (2 * G))]

        def prepare_b(i):
            return (permute_stream([(1, p, i // 2, i % 2 * (LANES // 2), LANES // 2) for p in range(3)])
                    + [P(permute_wo, 1, i)])

        def first_qkv(p):
            return [f for c in range(NCB) for f in qkv_chunk(o_s, 0, 0, p, c)]

        queue = ([[x_copy(0)]] + [[wa_copy(0, i)] for i in range(WCH)] + [[wa_copy(1, i)] for i in range(WCH)]
                 + [[wa_copy(2, i)] for i in range(WCH)] + [[x_copy(1)], [woa_copy(0)], [woa_copy(1)],
                                                            [x_copy(2)], b_copies(0)])
        pos = dict(started=0, waited=0)

        def start_up_to(k):
            while pos["started"] < min(k, len(queue)):
                for c in queue[pos["started"]]:
                    c.start()
                pos["started"] += 1

        def arrive():
            for c in queue[pos["waited"]]:
                c.wait()
            pos["waited"] += 1
            start_up_to(pos["waited"] + WINDOW)

        def arriving(p):
            return [f for i in range(WCH) for f in [arrive] + permute_stream([(0, p, i, 0, LANES)])]

        start_up_to(WINDOW)
        zero_halo(0)
        arrive()
        widen_x(0)
        _interleave(ln_stream(o_s, 0))
        _interleave(arriving(0))
        start_up_to(pos["waited"] + AHEAD)
        _interleave(first_qkv(0), arriving(1))
        start_up_to(pos["waited"] + AHEAD)
        _interleave(first_qkv(1), arriving(2))
        start_up_to(pos["waited"] + AHEAD)
        _interleave(first_qkv(2), [arrive, P(widen_x, 1)] + ln_stream(h_s, T) +
                    [f for i in range(2) for f in [arrive] + [P(permute_wo, 0, 4 * i + u) for u in range(4)]])
        start_up_to(len(queue))

        def step(first_layer, n, _):
            t0, lay0 = n % NT, n // NT
            t1, l1 = (n + 1) % NT, (n + 1) // NT
            t2 = (n + 2) % NT
            s0 = n % 2
            s1 = 1 - s0
            early, extra = [], []
            if first_layer:
                w0 = w1 = 0
                pl.when(n + 3 < NT)(lambda: x_copy(n + 3).start())
                for c in b_copies(n + 1):
                    c.start()
                pl.when(n + 2 < NT)(lambda: x_copy(n + 2).wait())
                for c in b_copies(n):
                    c.wait()
                early = [P(widen_x, jnp.minimum(n + 2, NT - 1), jnp.minimum(n + 2, NT))]
                extra = prepare_b(n)
            else:
                w0, w1 = lay0 % 2, l1 % 2
            qkv = [f for p in range(3) for c in range(NCB) for f in qkv_chunk(h_s, w1, s1, p, c)]
            k = int(len(qkv) * 0.95)
            qkv = qkv[:k] + [P(fill_halo, s1, t1 == 0)] + qkv[k:]
            k = int(len(qkv) * 0.9)
            _interleave(qkv[:k], attn_stream(s0, t0 * T)[0], early)
            _interleave(qkv[k:])
            wo = [f for c in range(NCB) for f in wo_chunk(w0, t0 * T, c, not first_layer)]
            k = int(len(wo) * 0.75)
            _interleave(wo[:k], ln_stream(h_s, t2 * T), extra)
            _interleave(wo[k:])
            if not first_layer:
                pl.when(lay0 == NL - 1)(lambda: out_copy(t0).start())

        lax.fori_loop(0, NT - 1, P(step, True), None)
        for c in b_copies(NT - 1):
            c.wait()
        _interleave(prepare_b(NT - 1))
        lax.fori_loop(NT - 1, NSTEP - 1, P(step, False), None)

        att, cuts = attn_stream((NSTEP - 1) % 2, (NT - 1) * T)
        cuts = [0] + cuts[len(cuts) // ESPLIT - 1::len(cuts) // ESPLIT]
        _interleave(att[:cuts[1]])
        for part in range(ESPLIT):
            _interleave([f for c in range(NCB) for f in wo_chunk((NL - 1) % 2, (NT - 1) * T, c, True, part, ESPLIT)],
                        att[cuts[part + 1]:cuts[part + 2]] if part + 1 < ESPLIT else [])
            out_copy(NT - 1, part, ESPLIT).start()
        for t in range(NT - 1):
            out_copy(t).wait()
        for part in range(ESPLIT):
            out_copy(NT - 1, part, ESPLIT).wait()

    scratch = [
        pltpu.VMEM((S, D), BF),
        pltpu.VMEM((NB, S + T, LANES), F32),
        pltpu.VMEM((2, D, 3 * D), BF),
        pltpu.VMEM((2, D, D), BF),
        pltpu.VMEM((2, 3, 7, D // 4, D // 2), I32),
        pltpu.VMEM((2, 7, D // 4, D // 2), I32),
        pltpu.VMEM((7, T // 4, D // 2), I32),
        pltpu.VMEM((7, T // 4, D // 2), I32),
        pltpu.VMEM((NB, T + 8, LANES), F32),
        pltpu.VMEM((NACC, 4, T // 2, LANES), F32),
        pltpu.VMEM((2, NB, T, LANES), F32),
        pltpu.VMEM((2, NB, T + HALO, LANES), F32),
        pltpu.VMEM((2, NB, T + HALO, LANES), F32),
        pltpu.SemaphoreType.DMA((NT,)),
        pltpu.SemaphoreType.DMA((3 * WCH,)),
        pltpu.SemaphoreType.DMA((2, 6)),
        pltpu.SemaphoreType.DMA((2,)),
        pltpu.SemaphoreType.DMA((NT - 1 + ESPLIT,)),
    ]
    return kernel, scratch


@jax.jit
def pallas_interleave_layers__sliding_local_dilated__sliding_local_dilated__prompt_kernel(
    A_x: jax.Array,
    A_wqkv: jax.Array,
    A_wo: jax.Array,
    B_x: jax.Array,
    B_wqkv: jax.Array,
    B_wo: jax.Array,
):
    del B_x
    kernel, scratch = make_kernel()
    any_spec = pl.BlockSpec(memory_space=pl.ANY)
    out = pl.pallas_call(
        kernel,
        out_shape=jax.ShapeDtypeStruct((S, D), BF),
        in_specs=[any_spec] * 5,
        out_specs=any_spec,
        scratch_shapes=scratch,
        compiler_params=pltpu.CompilerParams(vmem_limit_bytes=100 * 1024 * 1024),
    )(A_x.reshape(S, D), A_wqkv, A_wo, B_wqkv, B_wo)
    return out.reshape(1, S, D)
```
